```python
import os as _os
_os.environ.setdefault("JAX_PLATFORMS", "cpu")
import jax
import jax.numpy as jnp

def _softmax(x, axis=-1):
    return jax.nn.softmax(x, axis=axis)
def _gelu(x):
    return jax.nn.gelu(x, approximate=True)
def _silu(x):
    return jax.nn.silu(x)
def _sigmoid(x):
    return jax.nn.sigmoid(x)
def _layernorm(x, axis=-1, eps=1e-5):
    m = jnp.mean(x, axis=axis, keepdims=True)
    v = jnp.var(x, axis=axis, keepdims=True)
    return (x - m) / jnp.sqrt(v + eps)
def _scatter_add(tgt, idx, src, axis=0):
    return tgt.at[idx].add(src)
def _segment_sum(src, seg, n):
    return jax.ops.segment_sum(src, seg, n)
class _Rng:
    def __init__(self, key):
        self._k = key
    def _next(self):
        self._k, sub = jax.random.split(self._k)
        return sub
    def normal(self, shape):
        return jax.random.normal(self._next(), shape, dtype=jnp.bfloat16)
    def randint(self, lo, hi, shape):
        return jax.random.randint(self._next(), shape, lo, hi, dtype=jnp.int32)
    def uniform(self, shape, lo=0.0, hi=1.0):
        return jax.random.uniform(self._next(), shape, jnp.bfloat16, lo, hi)
    def permutation(self, n):
        return jax.random.permutation(self._next(), n)


kernel_name = 'concat_heads__mha_block_cached__mha_block_cached__near_ridge'

def setup_inputs():
    _rng = _Rng(jax.random.key(int.from_bytes(__import__("os").urandom(4), "little")))
    _w = (lambda a: (lambda t: t.astype(jnp.bfloat16) if jnp.issubdtype(t.dtype, jnp.floating) else t)(jnp.asarray(a)))
    def _A_setup():
        B, Sq, D = 8, 144, 640
        H, Sk, Dh = 32, 512, 128
        return {
            "x": _w((lambda *s: _rng.normal(s) * 0.8)(B, Sq, D)),
            "k_cache": _w((lambda *s: _rng.normal(s) * 0.8)(B, H, Sk, Dh)),
            "v_cache": _w((lambda *s: _rng.normal(s) * 0.05)(B, H, Sk, Dh)),
            "wq": _w((lambda *s: _rng.normal(s) * 0.8)(D, H * Dh) * (D ** -0.5)),
            "wo": _w((lambda *s: _rng.normal(s) * 0.05)(H * Dh, D) * ((H * Dh) ** -0.5)),
        }
    _A_in = _A_setup()

    def _B_setup():
        B, Sq, D = 8, 144, 640
        H, Sk, Dh = 32, 512, 128
        return {
            "x": _w((lambda *s: _rng.normal(s) * 0.8)(B, Sq, D)),
            "k_cache": _w((lambda *s: _rng.normal(s) * 0.8)(B, H, Sk, Dh)),
            "v_cache": _w((lambda *s: _rng.normal(s) * 0.05)(B, H, Sk, Dh)),
            "wq": _w((lambda *s: _rng.normal(s) * 0.8)(D, H * Dh) * (D ** -0.5)),
            "wo": _w((lambda *s: _rng.normal(s) * 0.05)(H * Dh, D) * ((H * Dh) ** -0.5)),
        }
    _B_in = _B_setup()

    return {
        "A_x": _A_in["x"],
        "A_k_cache": _A_in["k_cache"],
        "A_v_cache": _A_in["v_cache"],
        "A_wq": _A_in["wq"],
        "A_wo": _A_in["wo"],
        "B_x": _B_in["x"],
        "B_k_cache": _B_in["k_cache"],
        "B_v_cache": _B_in["v_cache"],
        "B_wq": _B_in["wq"],
        "B_wo": _B_in["wo"],
    }

def reference(A_x, A_k_cache, A_v_cache, A_wq, A_wo, B_x, B_k_cache, B_v_cache, B_wq, B_wo):
    def _A_ref(x, k_cache, v_cache, wq, wo):
        B, Sq, D = x.shape
        H, Dh = 32, 128
        q = (lambda x, *d: x.transpose(*d))((x @ wq).reshape(B, Sq, H, Dh), 0, 2, 1, 3)
        scores = jnp.einsum("bhqd,bhkd->bhqk", q, k_cache) * (Dh ** -0.5)
        p = _softmax(scores, axis=-1)
        o = jnp.einsum("bhqk,bhkd->bhqd", p, v_cache)
        return (lambda x, *d: x.transpose(*d))(o, 0, 2, 1, 3).reshape(B, Sq, H * Dh) @ wo

    def _B_ref(x, k_cache, v_cache, wq, wo):
        B, Sq, D = x.shape
        H, Dh = 32, 128
        q = (lambda x, *d: x.transpose(*d))((x @ wq).reshape(B, Sq, H, Dh), 0, 2, 1, 3)
        scores = jnp.einsum("bhqd,bhkd->bhqk", q, k_cache) * (Dh ** -0.5)
        p = _softmax(scores, axis=-1)
        o = jnp.einsum("bhqk,bhkd->bhqd", p, v_cache)
        return (lambda x, *d: x.transpose(*d))(o, 0, 2, 1, 3).reshape(B, Sq, H * Dh) @ wo

    a = _A_ref(A_x, A_k_cache, A_v_cache, A_wq, A_wo)
    b = _B_ref(B_x, B_k_cache, B_v_cache, B_wq, B_wo)
    return jnp.concatenate([a, b], axis=-1)
```

```python
import math

import jax
import jax.numpy as jnp
from jax import lax
from jax.experimental import pallas as pl
from jax.experimental.pallas import tpu as pltpu

B, SQ, D, H, SK, DH = 8, 144, 640, 32, 512, 128
G = 4
NG = H // G
R = SQ // 2
GW = G * DH
NJ = D // 128
NKV = 4
XS = ((0, 1), (1, 2), (3, 5))
QSCALE = float(DH ** -0.5 * math.log2(math.e))


def _bf16(x):
    return pltpu.bitcast(x, jnp.bfloat16)


def _u32(x):
    return pltpu.bitcast(x.astype(jnp.bfloat16), jnp.uint32)


def _kernel(xA, kA, vA, wqA, woA, xB, kB, vB, wqB, woB, out_hbm,
            x_buf, wq_buf, wo_buf, kv_buf, qA, qB, o_buf, acc, stage_o,
            sem_x, sem_wq, sem_kv, sem_w, sem_o):
    xA, kA, vA, wqA, woA, xB, kB, vB, wqB, woB, out_hbm = (
        r.bitcast(jnp.uint32)
        for r in (xA, kA, vA, wqA, woA, xB, kB, vB, wqB, woB, out_hbm))
    X, K, V, WQ, WO, Q = (xA, xB), (kA, kB), (vA, vB), (wqA, wqB), (woA, woB), (qA, qB)

    def mult(i, m):
        return i * m if isinstance(i, int) else pl.multiple_of(i * m, m)

    def slot_of(t):
        return t % NKV if isinstance(t, int) else jnp.bitwise_and(t, NKV - 1)

    def start_kv(s, g, slot):
        pltpu.make_async_copy(K[s].at[:, pl.ds(g * G, G)], kv_buf.at[slot, 0], sem_kv.at[slot]).start()
        pltpu.make_async_copy(V[s].at[:, pl.ds(g * G, G)], kv_buf.at[slot, 1], sem_kv.at[slot]).start()

    def wait_kv(slot):
        pltpu.make_async_copy(kv_buf.at[slot], kv_buf.at[slot], sem_kv.at[slot]).wait()

    def wq_copy(s, g, sem):
        return pltpu.make_async_copy(WQ[s].at[:, pl.ds(mult(g, GW), GW)], wq_buf.at[s, g], sem)

    def wo_copy(s, g, sem):
        return pltpu.make_async_copy(
            WO[s].at[pl.ds(mult(g, GW // 2), GW // 2), :], wo_buf.at[s, g], sem)

    def x_copy(s, b0, nb, sem):
        return pltpu.make_async_copy(X[s].at[pl.ds(b0, nb)], x_buf.at[s, pl.ds(b0, nb)], sem)

    def out_copy(s, b, j):
        return pltpu.make_async_copy(
            stage_o.at[s, j, pl.ds(b * R, R)],
            out_hbm.at[pl.ds(b * R, R), pl.ds(s * D + j * 128, 128)],
            sem_o.at[0])

    def qproj(s, g, b):
        q = jnp.dot(_bf16(x_buf[s, b]), _bf16(wq_buf[s, g]), preferred_element_type=jnp.float32)
        Q[s][g, b] = _u32(q * QSCALE)

    def qk(s, g, slot, b, h):
        q = _bf16(Q[s][g, b, :, h * DH:(h + 1) * DH])
        return lax.dot_general(q, _bf16(kv_buf[slot, 0, b, h]), (((1,), (1,)), ((), ())),
                               preferred_element_type=jnp.float32)

    def softmax(sc):
        m = jnp.max(sc, axis=-1, keepdims=True)
        p = jnp.exp2(sc - m)
        l = jnp.sum(p, axis=-1, keepdims=True)
        r = pltpu.reciprocal(l, approx=True)
        r = r * (2.0 - l * r)
        return p.astype(jnp.bfloat16), r

    def pv(slot, b, h, p, r):
        o = jnp.dot(p, _bf16(kv_buf[slot, 1, b, h]), preferred_element_type=jnp.float32)
        o_buf[b, :, h * DH:(h + 1) * DH] = _u32(o * r)

    def outproj(s, g, b):
        y = jnp.dot(_bf16(o_buf[b]), _bf16(wo_buf[s, g]), preferred_element_type=jnp.float32)
        v = jnp.where(g == 0, 0.0, acc[s, b]) + y
        acc[s, b] = v
        vu = _u32(v)
        for j in range(NJ):
            stage_o[s, j, pl.ds(b * R, R)] = vu[:, j * 128:(j + 1) * 128]
            pl.when(g == NG - 1)(lambda j=j: out_copy(s, b, j).start())

    def attention_step(s, g):
        slot = slot_of(g)
        for b in range(B):
            if s == 0:
                qproj(1, g, b)
            s0 = qk(s, g, slot, b, 0)
            if b > 0:
                outproj(s, g, b - 1)
            p0 = softmax(s0)
            s1 = qk(s, g, slot, b, 1)
            pv(slot, b, 0, *p0)
            p1 = softmax(s1)
            s2 = qk(s, g, slot, b, 2)
            pv(slot, b, 1, *p1)
            p2 = softmax(s2)
            s3 = qk(s, g, slot, b, 3)
            pv(slot, b, 2, *p2)
            p3 = softmax(s3)
            pv(slot, b, 3, *p3)
        outproj(s, g, B - 1)

    wq_copy(0, 0, sem_wq.at[0]).start()
    x_copy(0, *XS[0], sem_wq.at[0]).start()
    x_copy(0, *XS[1], sem_x.at[0]).start()
    wq_copy(0, 1, sem_wq.at[1]).start()
    x_copy(0, *XS[2], sem_x.at[1]).start()
    for g in range(2, NG):
        wq_copy(0, g, sem_wq.at[g]).start()
    for g in range(NKV):
        start_kv(0, g, g)
        if g == 0:
            x_copy(1, 0, B, sem_x.at[2]).start()
        wo_copy(0, g, sem_w.at[g]).start()
        wq_copy(1, g, sem_w.at[g]).start()
    for g in range(NKV, NG):
        wo_copy(0, g, sem_w.at[g]).start()
        wq_copy(1, g, sem_w.at[g]).start()
    for g in range(NG):
        wo_copy(1, g, sem_w.at[NG]).start()

    nb01 = XS[0][1] + XS[1][1]

    def phase1(i, carry):
        g0, g1 = 2 * i, 2 * i + 1
        first = i == 0
        wq_copy(0, g0, sem_wq.at[g0]).wait()
        pl.when(first)(lambda: x_copy(0, *XS[0], sem_wq.at[0]).wait())
        for b in range(XS[0][1]):
            qproj(0, g0, b)
        pl.when(first)(lambda: x_copy(0, *XS[1], sem_x.at[0]).wait())
        for b in range(XS[0][1], nb01):
            qproj(0, g0, b)
        wq_copy(0, g1, sem_wq.at[g1]).wait()
        for b in range(nb01):
            qproj(0, g1, b)
        pl.when(first)(lambda: x_copy(0, *XS[2], sem_x.at[1]).wait())
        for b in range(nb01, B):
            qproj(0, g0, b)
            qproj(0, g1, b)
        return carry

    lax.fori_loop(0, NG // 2, phase1, 0)
    x_copy(1, 0, B, sem_x.at[2]).wait()

    def phase2(g, carry):
        wait_kv(slot_of(g))
        wo_copy(0, g, sem_w.at[g]).wait()
        wq_copy(1, g, sem_w.at[g]).wait()
        attention_step(0, g)
        t = g + NKV
        pl.when(t < NG)(lambda: start_kv(0, t, slot_of(t)))
        pl.when(t >= NG)(lambda: start_kv(1, t - NG, slot_of(t)))
        return carry

    lax.fori_loop(0, NG, phase2, 0)
    for g in range(NG):
        wo_copy(1, g, sem_w.at[NG]).wait()

    def phase3(g, carry):
        wait_kv(slot_of(g))
        attention_step(1, g)
        t = g + NKV
        pl.when(t < NG)(lambda: start_kv(1, t, slot_of(t)))
        return carry

    lax.fori_loop(0, NG, phase3, 0)

    for s in range(2):
        for b in range(B):
            for j in range(NJ):
                out_copy(s, b, j).wait()


@jax.jit
def pallas_concat_heads__mha_block_cached__mha_block_cached__near_ridge_kernel(
    A_x: jax.Array,
    A_k_cache: jax.Array,
    A_v_cache: jax.Array,
    A_wq: jax.Array,
    A_wo: jax.Array,
    B_x: jax.Array,
    B_k_cache: jax.Array,
    B_v_cache: jax.Array,
    B_wq: jax.Array,
    B_wo: jax.Array,
):
    u32 = jnp.uint32
    scratch = [
        pltpu.VMEM((2, B, R, D), u32),
        pltpu.VMEM((2, NG, D // 2, GW), u32),
        pltpu.VMEM((2, NG, GW // 2, D), u32),
        pltpu.VMEM((NKV, 2, B, G, SK // 2, DH), u32),
        pltpu.VMEM((NG, B, R, GW), u32),
        pltpu.VMEM((NG, B, R, GW), u32),
        pltpu.VMEM((B, R, GW), u32),
        pltpu.VMEM((2, B, SQ, D), jnp.float32),
        pltpu.VMEM((2, NJ, B * R, 128), u32),
        pltpu.SemaphoreType.DMA((3,)),
        pltpu.SemaphoreType.DMA((NG,)),
        pltpu.SemaphoreType.DMA((NKV,)),
        pltpu.SemaphoreType.DMA((NG + 1,)),
        pltpu.SemaphoreType.DMA((1,)),
    ]
    out = pl.pallas_call(
        _kernel,
        out_shape=jax.ShapeDtypeStruct((B * SQ, 2 * D), jnp.bfloat16),
        in_specs=[pl.BlockSpec(memory_space=pl.ANY)] * 10,
        out_specs=pl.BlockSpec(memory_space=pl.ANY),
        scratch_shapes=scratch,
        compiler_params=pltpu.CompilerParams(
            vmem_limit_bytes=110 * 1024 * 1024,
            flags={"XLA_TPU_RESCHEDULE_DMA_DONES": True},
        ),
    )(A_x, A_k_cache, A_v_cache, A_wq, A_wo, B_x, B_k_cache, B_v_cache, B_wq, B_wo)
    return out.reshape(B, SQ, 2 * D)
```

```python
import math

import jax
import jax.numpy as jnp
from jax import lax
from jax.experimental import pallas as pl
from jax.experimental.pallas import tpu as pltpu

B, SQ, D, H, SK, DH = 8, 144, 640, 32, 512, 128
G = 4
NG = H // G
R = SQ // 2
GW = G * DH
NJ = D // 128
P1U = 4
NKV = 4
XS = ((0, 1), (1, 2), (3, 5))
QSCALE = float(DH ** -0.5 * math.log2(math.e))


def _bf16(x):
    return pltpu.bitcast(x, jnp.bfloat16)


def _u32(x):
    return pltpu.bitcast(x.astype(jnp.bfloat16), jnp.uint32)


def _kernel(xA, kA, vA, wqA, woA, xB, kB, vB, wqB, woB, out_hbm,
            x_buf, wq_buf, wo_buf, kv_buf, qA, qB, o_buf, acc, stage_o,
            sem_x, sem_wq, sem_kv, sem_w, sem_o):
    xA, kA, vA, wqA, woA, xB, kB, vB, wqB, woB, out_hbm = (
        r.bitcast(jnp.uint32)
        for r in (xA, kA, vA, wqA, woA, xB, kB, vB, wqB, woB, out_hbm))
    X, K, V, WQ, WO, Q = (xA, xB), (kA, kB), (vA, vB), (wqA, wqB), (woA, woB), (qA, qB)

    def mult(i, m):
        return i * m if isinstance(i, int) else pl.multiple_of(i * m, m)

    def slot_of(t):
        return t % NKV if isinstance(t, int) else jnp.bitwise_and(t, NKV - 1)

    def start_kv(s, g, slot):
        pltpu.make_async_copy(K[s].at[:, pl.ds(g * G, G)], kv_buf.at[slot, 0], sem_kv.at[slot]).start()
        pltpu.make_async_copy(V[s].at[:, pl.ds(g * G, G)], kv_buf.at[slot, 1], sem_kv.at[slot]).start()

    def wait_kv(slot):
        pltpu.make_async_copy(kv_buf.at[slot], kv_buf.at[slot], sem_kv.at[slot]).wait()

    def wq_copy(s, g, sem):
        return pltpu.make_async_copy(WQ[s].at[:, pl.ds(mult(g, GW), GW)], wq_buf.at[s, g], sem)

    def wo_copy(s, g, sem):
        return pltpu.make_async_copy(
            WO[s].at[pl.ds(mult(g, GW // 2), GW // 2), :], wo_buf.at[s, g], sem)

    def x_copy(s, b0, nb, sem):
        return pltpu.make_async_copy(X[s].at[pl.ds(b0, nb)], x_buf.at[s, pl.ds(b0, nb)], sem)

    def out_copy(s, b, j):
        return pltpu.make_async_copy(
            stage_o.at[s, j, pl.ds(b * R, R)],
            out_hbm.at[pl.ds(b * R, R), pl.ds(s * D + j * 128, 128)],
            sem_o.at[0])

    def qproj(s, g, b):
        q = jnp.dot(_bf16(x_buf[s, b]), _bf16(wq_buf[s, g]), preferred_element_type=jnp.float32)
        Q[s][g, b] = _u32(q * QSCALE)

    def qk(s, g, slot, b, h):
        q = _bf16(Q[s][g, b, :, h * DH:(h + 1) * DH])
        return lax.dot_general(q, _bf16(kv_buf[slot, 0, b, h]), (((1,), (1,)), ((), ())),
                               preferred_element_type=jnp.float32)

    def softmax(sc):
        m = jnp.max(sc, axis=-1, keepdims=True)
        p = jnp.exp2(sc - m)
        l = jnp.sum(p, axis=-1, keepdims=True)
        r = pltpu.reciprocal(l, approx=True)
        r = r * (2.0 - l * r)
        return p.astype(jnp.bfloat16), r

    def pv(slot, b, h, p, r):
        o = jnp.dot(p, _bf16(kv_buf[slot, 1, b, h]), preferred_element_type=jnp.float32)
        o_buf[b, :, h * DH:(h + 1) * DH] = _u32(o * r)

    def outproj(s, g, b):
        y = jnp.dot(_bf16(o_buf[b]), _bf16(wo_buf[s, g]), preferred_element_type=jnp.float32)
        v = jnp.where(g == 0, 0.0, acc[s, b]) + y
        acc[s, b] = v
        vu = _u32(v)
        for j in range(NJ):
            stage_o[s, j, pl.ds(b * R, R)] = vu[:, j * 128:(j + 1) * 128]
            pl.when(g == NG - 1)(lambda j=j: out_copy(s, b, j).start())

    def attention_step(s, g):
        slot = slot_of(g)
        for b in range(B):
            if s == 0:
                qproj(1, g, b)
            s0 = qk(s, g, slot, b, 0)
            if b > 0:
                outproj(s, g, b - 1)
            p0 = softmax(s0)
            s1 = qk(s, g, slot, b, 1)
            pv(slot, b, 0, *p0)
            p1 = softmax(s1)
            s2 = qk(s, g, slot, b, 2)
            pv(slot, b, 1, *p1)
            p2 = softmax(s2)
            s3 = qk(s, g, slot, b, 3)
            pv(slot, b, 2, *p2)
            p3 = softmax(s3)
            pv(slot, b, 3, *p3)
        outproj(s, g, B - 1)

    wq_copy(0, 0, sem_wq.at[0]).start()
    x_copy(0, *XS[0], sem_wq.at[0]).start()
    x_copy(0, *XS[1], sem_x.at[0]).start()
    wq_copy(0, 1, sem_wq.at[1]).start()
    x_copy(0, *XS[2], sem_x.at[1]).start()
    for g in range(2, NG):
        wq_copy(0, g, sem_wq.at[g]).start()
    for g in range(NKV):
        start_kv(0, g, g)
        if g == 0:
            x_copy(1, 0, B, sem_x.at[2]).start()
        wo_copy(0, g, sem_w.at[g]).start()
        wq_copy(1, g, sem_w.at[g]).start()
    for g in range(NKV, NG):
        wo_copy(0, g, sem_w.at[g]).start()
        wq_copy(1, g, sem_w.at[g]).start()
    for g in range(NG):
        wo_copy(1, g, sem_w.at[NG]).start()

    nb01 = XS[0][1] + XS[1][1]

    def phase1(i, carry):
        g0, g1 = P1U * i, P1U * i + 1
        first = i == 0
        wq_copy(0, g0, sem_wq.at[g0]).wait()
        pl.when(first)(lambda: x_copy(0, *XS[0], sem_wq.at[0]).wait())
        for b in range(XS[0][1]):
            qproj(0, g0, b)
        pl.when(first)(lambda: x_copy(0, *XS[1], sem_x.at[0]).wait())
        for b in range(XS[0][1], nb01):
            qproj(0, g0, b)
        wq_copy(0, g1, sem_wq.at[g1]).wait()
        for b in range(nb01):
            qproj(0, g1, b)
        pl.when(first)(lambda: x_copy(0, *XS[2], sem_x.at[1]).wait())
        for b in range(nb01, B):
            qproj(0, g0, b)
            qproj(0, g1, b)
        for u in range(2, P1U):
            wq_copy(0, g0 + u, sem_wq.at[g0 + u]).wait()
            for b in range(B):
                qproj(0, g0 + u, b)
        return carry

    lax.fori_loop(0, NG // P1U, phase1, 0)
    x_copy(1, 0, B, sem_x.at[2]).wait()

    def phase2(g, carry):
        wait_kv(slot_of(g))
        wo_copy(0, g, sem_w.at[g]).wait()
        wq_copy(1, g, sem_w.at[g]).wait()
        attention_step(0, g)
        t = g + NKV
        pl.when(t < NG)(lambda: start_kv(0, t, slot_of(t)))
        pl.when(t >= NG)(lambda: start_kv(1, t - NG, slot_of(t)))
        return carry

    lax.fori_loop(0, NG, phase2, 0)
    for g in range(NG):
        wo_copy(1, g, sem_w.at[NG]).wait()

    def phase3(g, carry):
        wait_kv(slot_of(g))
        attention_step(1, g)
        t = g + NKV
        pl.when(t < NG)(lambda: start_kv(1, t, slot_of(t)))
        return carry

    lax.fori_loop(0, NG, phase3, 0)

    for s in range(2):
        for b in range(B):
            for j in range(NJ):
                out_copy(s, b, j).wait()


@jax.jit
def pallas_concat_heads__mha_block_cached__mha_block_cached__near_ridge_kernel(
    A_x: jax.Array,
    A_k_cache: jax.Array,
    A_v_cache: jax.Array,
    A_wq: jax.Array,
    A_wo: jax.Array,
    B_x: jax.Array,
    B_k_cache: jax.Array,
    B_v_cache: jax.Array,
    B_wq: jax.Array,
    B_wo: jax.Array,
):
    u32 = jnp.uint32
    scratch = [
        pltpu.VMEM((2, B, R, D), u32),
        pltpu.VMEM((2, NG, D // 2, GW), u32),
        pltpu.VMEM((2, NG, GW // 2, D), u32),
        pltpu.VMEM((NKV, 2, B, G, SK // 2, DH), u32),
        pltpu.VMEM((NG, B, R, GW), u32),
        pltpu.VMEM((NG, B, R, GW), u32),
        pltpu.VMEM((B, R, GW), u32),
        pltpu.VMEM((2, B, SQ, D), jnp.float32),
        pltpu.VMEM((2, NJ, B * R, 128), u32),
        pltpu.SemaphoreType.DMA((3,)),
        pltpu.SemaphoreType.DMA((NG,)),
        pltpu.SemaphoreType.DMA((NKV,)),
        pltpu.SemaphoreType.DMA((NG + 1,)),
        pltpu.SemaphoreType.DMA((1,)),
    ]
    out = pl.pallas_call(
        _kernel,
        out_shape=jax.ShapeDtypeStruct((B * SQ, 2 * D), jnp.bfloat16),
        in_specs=[pl.BlockSpec(memory_space=pl.ANY)] * 10,
        out_specs=pl.BlockSpec(memory_space=pl.ANY),
        scratch_shapes=scratch,
        compiler_params=pltpu.CompilerParams(
            vmem_limit_bytes=110 * 1024 * 1024,
            flags={"XLA_TPU_RESCHEDULE_DMA_DONES": True},
        ),
    )(A_x, A_k_cache, A_v_cache, A_wq, A_wo, B_x, B_k_cache, B_v_cache, B_wq, B_wo)
    return out.reshape(B, SQ, 2 * D)
```

```python
import math

import jax
import jax.numpy as jnp
from jax import lax
from jax.experimental import pallas as pl
from jax.experimental.pallas import tpu as pltpu

B, SQ, D, H, SK, DH = 8, 144, 640, 32, 512, 128
G = 4
NG = H // G
R = SQ // 2
GW = G * DH
NJ = D // 128
NKV = 4
P1U = 4
XS = ((0, 1), (1, 1), (2, 1), (3, 2), (5, 3))
QSCALE = float(DH ** -0.5 * math.log2(math.e))


def _bf16(x):
    return pltpu.bitcast(x, jnp.bfloat16)


def _u32(x):
    return pltpu.bitcast(x.astype(jnp.bfloat16), jnp.uint32)


def _kernel(xA, kA, vA, wqA, woA, xB, kB, vB, wqB, woB, out_hbm,
            x_buf, wq_buf, wo_buf, kv_buf, qA, qB, o_buf, acc, stage_o,
            sem_x, sem_wq, sem_h, sem_kv, sem_w, sem_o):
    xA, kA, vA, wqA, woA, xB, kB, vB, wqB, woB, out_hbm = (
        r.bitcast(jnp.uint32)
        for r in (xA, kA, vA, wqA, woA, xB, kB, vB, wqB, woB, out_hbm))
    X, K, V, WQ, WO, Q = (xA, xB), (kA, kB), (vA, vB), (wqA, wqB), (woA, woB), (qA, qB)

    def mult(i, m):
        return i * m if isinstance(i, int) else pl.multiple_of(i * m, m)

    def slot_of(t):
        return t % NKV if isinstance(t, int) else jnp.bitwise_and(t, NKV - 1)

    def start_kv(s, g, slot):
        pltpu.make_async_copy(K[s].at[:, pl.ds(g * G, G)], kv_buf.at[slot, 0], sem_kv.at[slot]).start()
        pltpu.make_async_copy(V[s].at[:, pl.ds(g * G, G)], kv_buf.at[slot, 1], sem_kv.at[slot]).start()

    def wait_kv(slot):
        pltpu.make_async_copy(kv_buf.at[slot], kv_buf.at[slot], sem_kv.at[slot]).wait()

    def wq_copy(s, g, sem):
        return pltpu.make_async_copy(WQ[s].at[:, pl.ds(mult(g, GW), GW)], wq_buf.at[s, g], sem)

    def wq_half(g, hf, sem):
        return pltpu.make_async_copy(
            WQ[0].at[:, pl.ds(mult(2 * g + hf, GW // 2), GW // 2)],
            wq_buf.at[0, g, :, pl.ds(hf * (GW // 2), GW // 2)], sem)

    def wo_copy(s, g, sem):
        return pltpu.make_async_copy(
            WO[s].at[pl.ds(mult(g, GW // 2), GW // 2), :], wo_buf.at[s, g], sem)

    def x_copy(s, b0, nb, sem):
        return pltpu.make_async_copy(X[s].at[pl.ds(b0, nb)], x_buf.at[s, pl.ds(b0, nb)], sem)

    def xA_copy(c):
        return x_copy(0, *XS[c], sem_wq.at[0] if c == 0 else sem_x.at[c - 1])

    def xB_copy():
        return x_copy(1, 0, B, sem_x.at[len(XS) - 1])

    def out_copy(s, b, j):
        return pltpu.make_async_copy(
            stage_o.at[s, j, pl.ds(b * R, R)],
            out_hbm.at[pl.ds(b * R, R), pl.ds(s * D + j * 128, 128)],
            sem_o.at[0])

    def qproj(s, g, b):
        q = jnp.dot(_bf16(x_buf[s, b]), _bf16(wq_buf[s, g]), preferred_element_type=jnp.float32)
        Q[s][g, b] = _u32(q * QSCALE)

    def qproj_half(g, b, hf):
        cols = pl.ds(hf * (GW // 2), GW // 2)
        q = jnp.dot(_bf16(x_buf[0, b]), _bf16(wq_buf[0, g, :, cols]), preferred_element_type=jnp.float32)
        qA[g, b, :, cols] = _u32(q * QSCALE)

    def qk(s, g, slot, b, h):
        q = _bf16(Q[s][g, b, :, h * DH:(h + 1) * DH])
        return lax.dot_general(q, _bf16(kv_buf[slot, 0, b, h]), (((1,), (1,)), ((), ())),
                               preferred_element_type=jnp.float32)

    def softmax(sc):
        m = jnp.max(sc, axis=-1, keepdims=True)
        p = jnp.exp2(sc - m)
        l = jnp.sum(p, axis=-1, keepdims=True)
        r = pltpu.reciprocal(l, approx=True)
        r = r * (2.0 - l * r)
        return p.astype(jnp.bfloat16), r

    def pv(slot, b, h, p, r):
        o = jnp.dot(p, _bf16(kv_buf[slot, 1, b, h]), preferred_element_type=jnp.float32)
        o_buf[b, :, h * DH:(h + 1) * DH] = _u32(o * r)

    def outproj(s, g, b):
        y = jnp.dot(_bf16(o_buf[b]), _bf16(wo_buf[s, g]), preferred_element_type=jnp.float32)
        v = jnp.where(g == 0, 0.0, acc[s, b]) + y
        acc[s, b] = v
        vu = _u32(v)
        for j in range(NJ):
            stage_o[s, j, pl.ds(b * R, R)] = vu[:, j * 128:(j + 1) * 128]
            pl.when(g == NG - 1)(lambda j=j: out_copy(s, b, j).start())

    def attention_step(s, g):
        slot = slot_of(g)
        for b in range(B):
            if s == 0:
                qproj(1, g, b)
            s0 = qk(s, g, slot, b, 0)
            if b > 0:
                outproj(s, g, b - 1)
            p0 = softmax(s0)
            s1 = qk(s, g, slot, b, 1)
            pv(slot, b, 0, *p0)
            p1 = softmax(s1)
            s2 = qk(s, g, slot, b, 2)
            pv(slot, b, 1, *p1)
            p2 = softmax(s2)
            s3 = qk(s, g, slot, b, 3)
            pv(slot, b, 2, *p2)
            p3 = softmax(s3)
            pv(slot, b, 3, *p3)
        outproj(s, g, B - 1)

    wq_half(0, 0, sem_wq.at[0]).start()
    xA_copy(0).start()
    xA_copy(1).start()
    wq_half(0, 1, sem_h.at[0]).start()
    for c in range(2, len(XS)):
        xA_copy(c).start()
    for g in range(1, NG):
        if g % P1U == 0:
            wq_half(g, 0, sem_wq.at[g]).start()
            wq_half(g, 1, sem_h.at[g // P1U]).start()
        else:
            wq_copy(0, g, sem_wq.at[g]).start()
    for g in range(NKV):
        start_kv(0, g, g)
        if g == 0:
            xB_copy().start()
        wo_copy(0, g, sem_w.at[g]).start()
        wq_copy(1, g, sem_w.at[g]).start()
    for g in range(NKV, NG):
        wo_copy(0, g, sem_w.at[g]).start()
        wq_copy(1, g, sem_w.at[g]).start()
    for g in range(NG):
        wo_copy(1, g, sem_w.at[NG]).start()

    def phase1(i, carry):
        def wait_x(c):
            pl.when(i == 0)(lambda: xA_copy(c).wait())

        g = P1U * i
        wq_half(g, 0, sem_wq.at[g]).wait()
        wait_x(0)
        qproj_half(g, 0, 0)
        wait_x(1)
        qproj_half(g, 1, 0)
        wq_half(g, 1, sem_h.at[i]).wait()
        qproj_half(g, 0, 1)
        qproj_half(g, 1, 1)
        for c in range(2, len(XS)):
            wait_x(c)
            for b in range(XS[c][0], XS[c][0] + XS[c][1]):
                qproj(0, g, b)
        for u in range(1, P1U):
            wq_copy(0, g + u, sem_wq.at[g + u]).wait()
            for b in range(B):
                qproj(0, g + u, b)
        return carry

    lax.fori_loop(0, NG // P1U, phase1, 0)
    xB_copy().wait()

    def phase2(g, carry):
        wait_kv(slot_of(g))
        wo_copy(0, g, sem_w.at[g]).wait()
        wq_copy(1, g, sem_w.at[g]).wait()
        attention_step(0, g)
        t = g + NKV
        pl.when(t < NG)(lambda: start_kv(0, t, slot_of(t)))
        pl.when(t >= NG)(lambda: start_kv(1, t - NG, slot_of(t)))
        return carry

    lax.fori_loop(0, NG, phase2, 0)
    for g in range(NG):
        wo_copy(1, g, sem_w.at[NG]).wait()

    def phase3(g, carry):
        wait_kv(slot_of(g))
        attention_step(1, g)
        t = g + NKV
        pl.when(t < NG)(lambda: start_kv(1, t, slot_of(t)))
        return carry

    lax.fori_loop(0, NG, phase3, 0)

    for s in range(2):
        for b in range(B):
            for j in range(NJ):
                out_copy(s, b, j).wait()


assert XS[0] == (0, 1) and XS[1] == (1, 1) and sum(n for _, n in XS) == B


@jax.jit
def pallas_concat_heads__mha_block_cached__mha_block_cached__near_ridge_kernel(
    A_x: jax.Array,
    A_k_cache: jax.Array,
    A_v_cache: jax.Array,
    A_wq: jax.Array,
    A_wo: jax.Array,
    B_x: jax.Array,
    B_k_cache: jax.Array,
    B_v_cache: jax.Array,
    B_wq: jax.Array,
    B_wo: jax.Array,
):
    u32 = jnp.uint32
    scratch = [
        pltpu.VMEM((2, B, R, D), u32),
        pltpu.VMEM((2, NG, D // 2, GW), u32),
        pltpu.VMEM((2, NG, GW // 2, D), u32),
        pltpu.VMEM((NKV, 2, B, G, SK // 2, DH), u32),
        pltpu.VMEM((NG, B, R, GW), u32),
        pltpu.VMEM((NG, B, R, GW), u32),
        pltpu.VMEM((B, R, GW), u32),
        pltpu.VMEM((2, B, SQ, D), jnp.float32),
        pltpu.VMEM((2, NJ, B * R, 128), u32),
        pltpu.SemaphoreType.DMA((len(XS),)),
        pltpu.SemaphoreType.DMA((NG,)),
        pltpu.SemaphoreType.DMA((NG // P1U,)),
        pltpu.SemaphoreType.DMA((NKV,)),
        pltpu.SemaphoreType.DMA((NG + 1,)),
        pltpu.SemaphoreType.DMA((1,)),
    ]
    out = pl.pallas_call(
        _kernel,
        out_shape=jax.ShapeDtypeStruct((B * SQ, 2 * D), jnp.bfloat16),
        in_specs=[pl.BlockSpec(memory_space=pl.ANY)] * 10,
        out_specs=pl.BlockSpec(memory_space=pl.ANY),
        scratch_shapes=scratch,
        compiler_params=pltpu.CompilerParams(
            vmem_limit_bytes=110 * 1024 * 1024,
            flags={"XLA_TPU_RESCHEDULE_DMA_DONES": True},
        ),
    )(A_x, A_k_cache, A_v_cache, A_wq, A_wo, B_x, B_k_cache, B_v_cache, B_wq, B_wo)
    return out.reshape(B, SQ, 2 * D)
```

```python
import math

import jax
import jax.numpy as jnp
from jax import lax
from jax.experimental import pallas as pl
from jax.experimental.pallas import tpu as pltpu

B, SQ, D, H, SK, DH = 8, 144, 640, 32, 512, 128
G = 4
NG = H // G
R = SQ // 2
GW = G * DH
NJ = D // 128
NKV = 4
P1U = 4
XS = ((0, 1), (1, 1), (2, 1), (3, 2), (5, 3))
QSCALE = float(DH ** -0.5 * math.log2(math.e))


def _bf16(x):
    return pltpu.bitcast(x, jnp.bfloat16)


def _u32(x):
    return pltpu.bitcast(x.astype(jnp.bfloat16), jnp.uint32)


def _kernel(*refs):
    pl.run_scoped(
        lambda *sems: _body(*refs, *sems),
        pltpu.SemaphoreType.DMA((len(XS),)),
        pltpu.SemaphoreType.DMA((NG,)),
        pltpu.SemaphoreType.DMA((NG // P1U,)),
        pltpu.SemaphoreType.DMA((NKV,)),
        pltpu.SemaphoreType.DMA((NG + 1,)),
        pltpu.SemaphoreType.DMA((1,)),
    )


def _body(xA, kA, vA, wqA, woA, xB, kB, vB, wqB, woB, out_hbm,
          x_buf, wq_buf, wo_buf, kv_buf, qA, qB, o_buf, acc, stage_o,
          sem_x, sem_wq, sem_h, sem_kv, sem_w, sem_o):
    xA, kA, vA, wqA, woA, xB, kB, vB, wqB, woB, out_hbm = (
        r.bitcast(jnp.uint32)
        for r in (xA, kA, vA, wqA, woA, xB, kB, vB, wqB, woB, out_hbm))
    X, K, V, WQ, WO, Q = (xA, xB), (kA, kB), (vA, vB), (wqA, wqB), (woA, woB), (qA, qB)

    def mult(i, m):
        return i * m if isinstance(i, int) else pl.multiple_of(i * m, m)

    def slot_of(t):
        return t % NKV if isinstance(t, int) else jnp.bitwise_and(t, NKV - 1)

    def start_kv(s, g, slot):
        pltpu.make_async_copy(K[s].at[:, pl.ds(g * G, G)], kv_buf.at[slot, 0], sem_kv.at[slot]).start()
        pltpu.make_async_copy(V[s].at[:, pl.ds(g * G, G)], kv_buf.at[slot, 1], sem_kv.at[slot]).start()

    def wait_kv(slot):
        pltpu.make_async_copy(kv_buf.at[slot], kv_buf.at[slot], sem_kv.at[slot]).wait()

    def wq_copy(s, g, sem):
        return pltpu.make_async_copy(WQ[s].at[:, pl.ds(mult(g, GW), GW)], wq_buf.at[s, g], sem)

    def wq_half(g, hf, sem):
        return pltpu.make_async_copy(
            WQ[0].at[:, pl.ds(mult(2 * g + hf, GW // 2), GW // 2)],
            wq_buf.at[0, g, :, pl.ds(hf * (GW // 2), GW // 2)], sem)

    def wo_copy(s, g, sem):
        return pltpu.make_async_copy(
            WO[s].at[pl.ds(mult(g, GW // 2), GW // 2), :], wo_buf.at[s, g], sem)

    def x_copy(s, b0, nb, sem):
        return pltpu.make_async_copy(X[s].at[pl.ds(b0, nb)], x_buf.at[s, pl.ds(b0, nb)], sem)

    def xA_copy(c):
        return x_copy(0, *XS[c], sem_wq.at[0] if c == 0 else sem_x.at[c - 1])

    def xB_copy():
        return x_copy(1, 0, B, sem_x.at[len(XS) - 1])

    def out_copy(s, b, j):
        return pltpu.make_async_copy(
            stage_o.at[s, j, pl.ds(b * R, R)],
            out_hbm.at[pl.ds(b * R, R), pl.ds(s * D + j * 128, 128)],
            sem_o.at[0])

    def qproj(s, g, b):
        q = jnp.dot(_bf16(x_buf[s, b]), _bf16(wq_buf[s, g]), preferred_element_type=jnp.float32)
        Q[s][g, b] = _u32(q * QSCALE)

    def qproj_half(g, b, hf):
        cols = pl.ds(hf * (GW // 2), GW // 2)
        q = jnp.dot(_bf16(x_buf[0, b]), _bf16(wq_buf[0, g, :, cols]), preferred_element_type=jnp.float32)
        qA[g, b, :, cols] = _u32(q * QSCALE)

    def qk(s, g, slot, b, h):
        q = _bf16(Q[s][g, b, :, h * DH:(h + 1) * DH])
        return lax.dot_general(q, _bf16(kv_buf[slot, 0, b, h]), (((1,), (1,)), ((), ())),
                               preferred_element_type=jnp.float32)

    def softmax(sc):
        m = jnp.max(sc, axis=-1, keepdims=True)
        p = jnp.exp2(sc - m)
        l = jnp.sum(p, axis=-1, keepdims=True)
        r = pltpu.reciprocal(l, approx=True)
        r = r * (2.0 - l * r)
        return p.astype(jnp.bfloat16), r

    def pv(slot, b, h, p, r):
        o = jnp.dot(p, _bf16(kv_buf[slot, 1, b, h]), preferred_element_type=jnp.float32)
        o_buf[b, :, h * DH:(h + 1) * DH] = _u32(o * r)

    def outproj(s, g, b):
        y = jnp.dot(_bf16(o_buf[b]), _bf16(wo_buf[s, g]), preferred_element_type=jnp.float32)
        v = jnp.where(g == 0, 0.0, acc[s, b]) + y
        acc[s, b] = v
        vu = _u32(v)
        for j in range(NJ):
            stage_o[s, j, pl.ds(b * R, R)] = vu[:, j * 128:(j + 1) * 128]
            pl.when(g == NG - 1)(lambda j=j: out_copy(s, b, j).start())

    def attention_step(s, g):
        slot = slot_of(g)
        for b in range(B):
            if s == 0:
                qproj(1, g, b)
            s0 = qk(s, g, slot, b, 0)
            if b > 0:
                outproj(s, g, b - 1)
            p0 = softmax(s0)
            s1 = qk(s, g, slot, b, 1)
            pv(slot, b, 0, *p0)
            p1 = softmax(s1)
            s2 = qk(s, g, slot, b, 2)
            pv(slot, b, 1, *p1)
            p2 = softmax(s2)
            s3 = qk(s, g, slot, b, 3)
            pv(slot, b, 2, *p2)
            p3 = softmax(s3)
            pv(slot, b, 3, *p3)
        outproj(s, g, B - 1)

    wq_half(0, 0, sem_wq.at[0]).start()
    xA_copy(0).start()
    xA_copy(1).start()
    wq_half(0, 1, sem_h.at[0]).start()
    for c in range(2, len(XS)):
        xA_copy(c).start()
    for g in range(1, NG):
        if g % P1U == 0:
            wq_half(g, 0, sem_wq.at[g]).start()
            wq_half(g, 1, sem_h.at[g // P1U]).start()
        else:
            wq_copy(0, g, sem_wq.at[g]).start()
    for g in range(NKV):
        start_kv(0, g, g)
        if g == 0:
            xB_copy().start()
        wo_copy(0, g, sem_w.at[g]).start()
        wq_copy(1, g, sem_w.at[g]).start()
    for g in range(NKV, NG):
        wo_copy(0, g, sem_w.at[g]).start()
        wq_copy(1, g, sem_w.at[g]).start()
    for g in range(NG):
        wo_copy(1, g, sem_w.at[NG]).start()

    def phase1(i, carry):
        def wait_x(c):
            pl.when(i == 0)(lambda: xA_copy(c).wait())

        g = P1U * i
        wq_half(g, 0, sem_wq.at[g]).wait()
        wait_x(0)
        qproj_half(g, 0, 0)
        wait_x(1)
        qproj_half(g, 1, 0)
        wq_half(g, 1, sem_h.at[i]).wait()
        qproj_half(g, 0, 1)
        qproj_half(g, 1, 1)
        for c in range(2, len(XS)):
            wait_x(c)
            for b in range(XS[c][0], XS[c][0] + XS[c][1]):
                qproj(0, g, b)
        for u in range(1, P1U):
            wq_copy(0, g + u, sem_wq.at[g + u]).wait()
            for b in range(B):
                qproj(0, g + u, b)
        return carry

    lax.fori_loop(0, NG // P1U, phase1, 0)
    xB_copy().wait()

    def phase2(g, carry):
        wait_kv(slot_of(g))
        wo_copy(0, g, sem_w.at[g]).wait()
        wq_copy(1, g, sem_w.at[g]).wait()
        attention_step(0, g)
        t = g + NKV
        pl.when(t < NG)(lambda: start_kv(0, t, slot_of(t)))
        pl.when(t >= NG)(lambda: start_kv(1, t - NG, slot_of(t)))
        return carry

    lax.fori_loop(0, NG, phase2, 0)
    for g in range(NG):
        wo_copy(1, g, sem_w.at[NG]).wait()

    def phase3(g, carry):
        wait_kv(slot_of(g))
        attention_step(1, g)
        t = g + NKV
        pl.when(t < NG)(lambda: start_kv(1, t, slot_of(t)))
        return carry

    lax.fori_loop(0, NG, phase3, 0)

    for s in range(2):
        for b in range(B):
            for j in range(NJ):
                out_copy(s, b, j).wait()


assert XS[0] == (0, 1) and XS[1] == (1, 1) and sum(n for _, n in XS) == B


@jax.jit
def pallas_concat_heads__mha_block_cached__mha_block_cached__near_ridge_kernel(
    A_x: jax.Array,
    A_k_cache: jax.Array,
    A_v_cache: jax.Array,
    A_wq: jax.Array,
    A_wo: jax.Array,
    B_x: jax.Array,
    B_k_cache: jax.Array,
    B_v_cache: jax.Array,
    B_wq: jax.Array,
    B_wo: jax.Array,
):
    u32 = jnp.uint32
    scratch = [
        pltpu.VMEM((2, B, R, D), u32),
        pltpu.VMEM((2, NG, D // 2, GW), u32),
        pltpu.VMEM((2, NG, GW // 2, D), u32),
        pltpu.VMEM((NKV, 2, B, G, SK // 2, DH), u32),
        pltpu.VMEM((NG, B, R, GW), u32),
        pltpu.VMEM((NG, B, R, GW), u32),
        pltpu.VMEM((B, R, GW), u32),
        pltpu.VMEM((2, B, SQ, D), jnp.float32),
        pltpu.VMEM((2, NJ, B * R, 128), u32),
    ]
    out = pl.pallas_call(
        _kernel,
        out_shape=jax.ShapeDtypeStruct((B * SQ, 2 * D), jnp.bfloat16),
        in_specs=[pl.BlockSpec(memory_space=pl.ANY)] * 10,
        out_specs=pl.BlockSpec(memory_space=pl.ANY),
        scratch_shapes=scratch,
        compiler_params=pltpu.CompilerParams(
            vmem_limit_bytes=110 * 1024 * 1024,
            flags={"XLA_TPU_RESCHEDULE_DMA_DONES": True},
        ),
    )(A_x, A_k_cache, A_v_cache, A_wq, A_wo, B_x, B_k_cache, B_v_cache, B_wq, B_wo)
    return out.reshape(B, SQ, 2 * D)
```
